```python
import jax
import jax.numpy as jnp

def _softmax(x, axis=-1):
    return jax.nn.softmax(x, axis=axis)
def _gelu(x):
    return jax.nn.gelu(x, approximate=True)
def _silu(x):
    return jax.nn.silu(x)
def _sigmoid(x):
    return jax.nn.sigmoid(x)
def _layernorm(x, axis=-1, eps=1e-5):
    m = jnp.mean(x, axis=axis, keepdims=True)
    v = jnp.var(x, axis=axis, keepdims=True)
    return (x - m) / jnp.sqrt(v + eps)
def _scatter_add(tgt, idx, src, axis=0):
    return tgt.at[idx].add(src)
def _segment_sum(src, seg, n):
    return jax.ops.segment_sum(src, seg, n)
class _Rng:
    def __init__(self, key):
        self._k = key
    def _next(self):
        self._k, sub = jax.random.split(self._k)
        return sub
    def normal(self, shape):
        return jax.random.normal(self._next(), shape, dtype=jnp.bfloat16)
    def randint(self, lo, hi, shape):
        return jax.random.randint(self._next(), shape, lo, hi, dtype=jnp.int32)
    def uniform(self, shape, lo=0.0, hi=1.0):
        return jax.random.uniform(self._next(), shape, jnp.bfloat16, lo, hi)
    def permutation(self, n):
        return jax.random.permutation(self._next(), n)


kernel_name = 'standalone__structured_sparse_n_m__ragged'

def setup_inputs():
    _rng = _Rng(jax.random.key(int.from_bytes(__import__("os").urandom(4), "little")))
    _w = (lambda a: (lambda t: t.astype(jnp.bfloat16) if jnp.issubdtype(t.dtype, jnp.floating) else t)(jnp.asarray(a)))
    B, S, D = 16, 4096, 576
    assert D % 4 == 0, "d_model must be divisible by M=4 for 2:4 sparsity"
    return {
        "x": _w((lambda *s: _rng.normal(s) * 0.05)(B, S, D)),
        "w": _w((lambda *s: _rng.normal(s) * 0.05)(D, D)),
        "b": _w((lambda *s: _rng.normal(s) * 0.05)(D)),
    }

def reference(x, w, b):
    B, S, D = x.shape
    N, M = 2, 4
    G = D // M
    wg = w.reshape(G, M, D)
    mag = jnp.abs(wg)
    order = jnp.argsort(mag, 1)
    thr = jnp.take_along_axis(mag, order[:, M - N:M - N + 1, :], 1)
    mask = (lambda x, dt: x.astype(dt))(mag >= thr, w.dtype)
    wp = (wg * mask).reshape(D, D)
    return jnp.einsum("bsd,df->bsf", x, wp) + b
```

```python
import numpy as np

import jax
import jax.numpy as jnp
from jax import lax
import jax.experimental.pallas as pl
import jax.experimental.pallas.tpu as pltpu

D = 576
QW = 1024
NQ = 64
NI = 32
NB = 3
NA0, NA1 = 2, 2
NINIT = 12
MAXI = (12, 16)
F32, BF16, I32 = jnp.float32, jnp.bfloat16, jnp.int32

AT = {0: [(0, 1), (3, 1)], 1: [(2, 1), (3, 1)], 2: [(0, 1)], 3: [(3, 1)],
      4: [(0, 1), (1, 1)], 5: [(2, 1), (0, -1)], 6: [(1, 1), (3, -1)]}
BT = {0: [(0, 1), (3, 1)], 1: [(0, 1)], 2: [(1, 1), (3, -1)], 3: [(2, 1), (0, -1)],
      4: [(3, 1)], 5: [(0, 1), (1, 1)], 6: [(2, 1), (3, 1)]}
CT = {0: [(0, 1), (3, 1)], 1: [(2, 1), (3, -1)], 2: [(1, 1), (3, 1)], 3: [(0, 1), (2, 1)],
      4: [(0, -1), (1, 1)], 5: [(3, 1)], 6: [(0, 1)]}
NT = (4, 2, 2, 4)
ORDER1 = (3, 4, 2, 1, 6, 0, 5)
ORDER2 = (5, 1, 2, 4, 3, 0, 6)
TAIL_AT = {0: -1, 1: 2, 2: 3, 3: -1}


def _dma_plan():
    nb = (NQ - NA0 - NA1) // NB
    qs = list(range(NA0)) + [NA0 + NB * i for i in range(nb)]
    qs += [NQ - NA1 + i for i in range(NA1)] + [NQ]
    rounds = len(qs) - 1
    w1, r2, w2 = 6, 10, 16
    rn, wn, tab = NINIT, 0, []
    for j in range(rounds):
        mx = MAXI[0] if (j < NA0 or j >= NA0 + nb) else MAXI[1]
        want_r = 10 if j < 2 else (16 if j >= r2 else 0)
        want_w = 16 if (w1 <= j <= r2 or j >= w2) else 0
        assert rn >= qs[j + 1]
        nr = max(0, min(want_r, mx, NQ - rn, qs[min(j + 2, rounds)] + NI - rn))
        nw = min(want_w, mx, qs[j] - wn)
        tab += [rn, nr, wn, nw]
        rn += nr
        wn += nw
    assert rn == NQ and wn == NQ - 1
    return tab


def _comb(terms, get):
    v = get(terms[0][0])
    for q, s in terms[1:]:
        v = v + get(q) if s > 0 else v - get(q)
    return v


def _quadrants(a):
    h, w = a.shape[0] // 2, a.shape[1] // 2
    return a[:h, :w], a[:h, w:], a[h:, :w], a[h:, w:]


def _pack(a):
    return pltpu.bitcast(a.astype(BF16), I32)


def _unpack(a):
    return pltpu.bitcast(a, BF16)


class _Acc:
    def __init__(self, n):
        self.left, self.pos, self.neg = n, None, None

    def add(self, s, v):
        self.left -= 1
        if self.pos is not None:
            self.pos = self.pos + v if s > 0 else self.pos - v
        elif s > 0:
            self.pos = v if self.neg is None else v - self.neg
        else:
            self.neg = v if self.neg is None else self.neg + v
        return self.left == 0


def _prepare(w_ref, b_ref, wf_ref, sa_ref, wtail_ref, bias_ref):
    brow = b_ref[...].astype(F32).reshape(1, D)
    for j in range(5):
        if j < 4:
            blk = w_ref[:, 128 * j:128 * j + 128].astype(F32)
            bj = brow[:, 128 * j:128 * j + 128]
        else:
            blk = jnp.concatenate(
                [w_ref[:, 512:D].astype(F32), jnp.zeros((D, 64), F32)], axis=1)
            bj = jnp.concatenate([brow[:, 512:D], jnp.zeros((1, 64), F32)], axis=1)
        wf_ref[j, 0:D] = blk
        wf_ref[j, D:640] = jnp.broadcast_to(bj, (640 - D, 128))
    for j in range(5):
        v = [wf_ref[j, pl.ds(i, D // 4, stride=4), :] for i in range(4)]
        m = [jnp.abs(a) for a in v]
        hi1, lo1 = jnp.maximum(m[0], m[1]), jnp.minimum(m[0], m[1])
        hi2, lo2 = jnp.maximum(m[2], m[3]), jnp.minimum(m[2], m[3])
        thr = jnp.maximum(jnp.minimum(hi1, hi2), jnp.maximum(lo1, lo2))
        for i in range(4):
            wf_ref[j, pl.ds(i, D // 4, stride=4), :] = v[i] * (m[i] >= thr).astype(F32)
    wt = jnp.concatenate(
        [wf_ref[j].T if j < 4 else wf_ref[j].T[:64] for j in range(5)], axis=0)
    last = wt[:, 512:640]
    low = lax.broadcasted_iota(I32, last.shape, 1) < 64
    bias_ref[...] = jnp.where(low, pltpu.roll(last, 64, 1), last)
    wtail_ref[...] = _pack(last)
    a0 = _quadrants(wt[:, 0:512])
    for r in range(7):
        a1 = _quadrants(_comb(AT[r], lambda q: a0[q]))
        for t in range(7):
            sa_ref[7 * r + t] = _pack(_comb(AT[t], lambda u: a1[u]))


def _group(x_ref, o_ref, c0, nxt, first, pend, sa_ref, wtail_ref, bias_ref):
    def direct(r, t):
        return len(BT[r]) == 1 and len(BT[t]) == 1

    def tile(ref, c, q, u):
        k, j = 2 * (q // 2) + u // 2, 2 * (q % 2) + u % 2
        return ref[128 * k:128 * k + 128, pl.ds(c + 128 * j, 128)]

    def xop(r, ref, c):
        cache = {}

        def gx(q, u):
            if (q, u) not in cache:
                cache[(q, u)] = tile(ref, c, q, u).astype(F32)
            return cache[(q, u)]

        b1 = [_comb(BT[r], lambda q: gx(q, u)) for u in range(4)]
        for t in range(7):
            if not direct(r, t):
                pend[t] = _comb(BT[t], lambda u: b1[u]).astype(BF16)

    acc = {(q, u): _Acc(NT[q] + 1) for q in range(4) for u in range(4)}

    def put(q, u, s, v):
        if acc[(q, u)].add(s, v):
            r0 = 288 * (q // 2) + 144 * (u // 2)
            cc = 256 * (q % 2) + 128 * (u % 2)
            o_ref[r0:r0 + 144, pl.ds(c0 + cc, 128)] = acc[(q, u)].pos.astype(BF16)

    def tails(pos):
        for j, p in TAIL_AT.items():
            if p == pos:
                t = jnp.dot(_unpack(wtail_ref[...])[:, 0:64],
                            x_ref[512:D, pl.ds(c0 + 128 * j, 128)],
                            preferred_element_type=F32) + bias_ref[...]
                for i in range(4):
                    put(2 * (i // 2) + j // 2, 2 * (i % 2) + j % 2, 1, t[144 * i:144 * i + 144])

    if first:
        xop(ORDER1[0], x_ref, c0)
    tails(-1)
    for pos, r in enumerate(ORDER1):
        c = [_Acc(NT[u]) for u in range(4)]
        for t in ORDER2:
            sb = tile(x_ref, c0, BT[r][0][0], BT[t][0][0]) if direct(r, t) else pend.pop(t)
            m = jnp.dot(_unpack(sa_ref[7 * r + t]), sb, preferred_element_type=F32)
            for u, s in CT[t]:
                if c[u].add(s, m):
                    for q, s1 in CT[r]:
                        put(q, u, s1, c[u].pos)
        if pos + 1 < 7:
            xop(ORDER1[pos + 1], x_ref, c0)
        elif nxt is not None:
            xop(ORDER1[0], nxt[0], nxt[2])
        tails(pos)


def _kernel(x_hbm, w_hbm, b_hbm, o_hbm, xbuf, obuf, w_ref, b_ref, wf_ref, sa_ref,
            wtail_ref, bias_ref, tab, rsem, wsem, csem):
    def rd(q):
        s = q & (NI - 1)
        src = x_hbm.at[q >> 2, :, pl.ds(pl.multiple_of((q & 3) * QW, QW), QW)]
        return pltpu.make_async_copy(src, xbuf.at[s], rsem.at[s])

    def wr(q, c0):
        dst = o_hbm.at[q >> 2, :, pl.ds(pl.multiple_of((q & 3) * QW + c0, 256), 256)]
        return pltpu.make_async_copy(obuf.at[q, :, pl.ds(c0, 256)], dst, wsem.at[0])

    cw = pltpu.make_async_copy(w_hbm, w_ref, csem.at[0])
    cb = pltpu.make_async_copy(b_hbm, b_ref, csem.at[1])
    cw.start()
    cb.start()
    rd(0).start()
    for i, v in enumerate(_dma_plan()):
        tab[i] = v
    cw.wait()
    cb.wait()
    _prepare(w_ref, b_ref, wf_ref, sa_ref, wtail_ref, bias_ref)
    for q in range(1, NINIT):
        rd(q).start()

    def rnd(nq, nmax):
        def body(_, carry):
            j, q = carry
            for k in range(nq):
                rd(q + k).wait()
            r0, nr, w0, nw = tab[4 * j], tab[4 * j + 1], tab[4 * j + 2], tab[4 * j + 3]
            for t in range(nmax):
                for c0 in range(0, QW, 256):
                    @pl.when(t < nw)
                    def _():
                        wr(jnp.minimum(w0 + t, NQ - 1), c0).start()
            gs = [(xbuf.at[(q + k) & (NI - 1)], obuf.at[q + k], c0)
                  for k in range(nq) for c0 in range(0, QW, 512)]
            pend = {}
            for gi, (xv, ov, c0) in enumerate(gs):
                nxt = gs[gi + 1] if gi + 1 < len(gs) else None
                _group(xv, ov, c0, nxt, gi == 0, pend, sa_ref, wtail_ref, bias_ref)
            for t in range(nmax):
                @pl.when(t < nr)
                def _():
                    rd(jnp.minimum(r0 + t, NQ - 1)).start()
            return j + 1, q + nq
        return body

    def phase(ph, carry):
        carry = lax.fori_loop(0, jnp.where(ph == 0, NA0, NA1), rnd(1, MAXI[0]), carry)
        nb = (NQ - NA0 - NA1) // NB
        return lax.fori_loop(0, jnp.where(ph == 0, nb, 0), rnd(NB, MAXI[1]), carry)

    lax.fori_loop(0, 2, phase, (jnp.int32(0), jnp.int32(0)))
    for c0 in range(0, QW, 256):
        wr(NQ - 1, c0).start()
    pltpu.make_async_copy(obuf, obuf, wsem.at[0]).wait()


@jax.jit
def pallas_standalone__structured_sparse_n_m__ragged_kernel(
    x: jax.Array,
    w: jax.Array,
    b: jax.Array,
):
    B, S, _ = x.shape
    assert x.shape == (16, 4096, D) and w.shape == (D, D) and b.shape == (D,)
    any_spec = pl.BlockSpec(memory_space=pl.ANY)
    out_t = pl.pallas_call(
        _kernel,
        in_specs=[any_spec] * 3,
        out_specs=any_spec,
        out_shape=jax.ShapeDtypeStruct((B, D, S), x.dtype),
        scratch_shapes=[
            pltpu.VMEM((NI, D, QW), BF16),
            pltpu.VMEM((NQ, D, QW), BF16),
            pltpu.VMEM((D, D), BF16),
            pltpu.VMEM((D,), BF16),
            pltpu.VMEM((5, 640, 128), F32),
            pltpu.VMEM((49, 72, 128), I32),
            pltpu.VMEM((D // 2, 128), I32),
            pltpu.VMEM((D, 128), F32),
            pltpu.SMEM((len(_dma_plan()),), I32),
            pltpu.SemaphoreType.DMA((NI,)),
            pltpu.SemaphoreType.DMA((1,)),
            pltpu.SemaphoreType.DMA((2,)),
        ],
        compiler_params=pltpu.CompilerParams(
            vmem_limit_bytes=124 * 1024 * 1024, disable_bounds_checks=True),
    )(jnp.swapaxes(x, 1, 2), w, b)
    return jnp.swapaxes(out_t, 1, 2)
```

```python
import numpy as np

import jax
import jax.numpy as jnp
from jax import lax
import jax.experimental.pallas as pl
import jax.experimental.pallas.tpu as pltpu

D = 576
QW = 1024
NQ = 64
NI = 32
NB = 5
NA0, NA1 = 4, 5
NINIT = 12
MAX_RD = (12, 16)
MAX_WR = (12, 16)
MAX_MID = 12
F32, BF16, I32 = jnp.float32, jnp.bfloat16, jnp.int32

AT = {0: [(0, 1), (3, 1)], 1: [(2, 1), (3, 1)], 2: [(0, 1)], 3: [(3, 1)],
      4: [(0, 1), (1, 1)], 5: [(2, 1), (0, -1)], 6: [(1, 1), (3, -1)]}
BT = {0: [(0, 1), (3, 1)], 1: [(0, 1)], 2: [(1, 1), (3, -1)], 3: [(2, 1), (0, -1)],
      4: [(3, 1)], 5: [(0, 1), (1, 1)], 6: [(2, 1), (3, 1)]}
CT = {0: [(0, 1), (3, 1)], 1: [(2, 1), (3, -1)], 2: [(1, 1), (3, 1)], 3: [(0, 1), (2, 1)],
      4: [(0, -1), (1, 1)], 5: [(3, 1)], 6: [(0, 1)]}
NT = (4, 2, 2, 4)
ORDER1 = (3, 4, 2, 1, 6, 0, 5)
ORDER2 = (5, 1, 2, 4, 3, 0, 6)
TAIL_AT = {0: -1, 1: 2, 2: 3, 3: -1}


def _dma_plan():
    nb = (NQ - NA0 - NA1) // NB
    qs = list(range(NA0)) + [NA0 + NB * i for i in range(nb)]
    qs += [NQ - NA1 + i for i in range(NA1)] + [NQ]
    rounds = len(qs) - 1
    first_reads = (10, 8)
    w1, w1_end, r2, w2 = 12, 15, 7, 22
    assert NINIT <= NI
    rn, wn, tab = NINIT, 0, []
    for j in range(rounds):
        short = j < NA0 or j >= NA0 + nb
        want = first_reads[j] if j < len(first_reads) else (NQ if j >= r2 else 0)
        assert rn >= qs[j + 1]
        nr = max(0, min(want, MAX_RD[1 - short], NQ - rn, qs[j + 1] + NI - rn))
        assert rn + nr <= qs[j + 1] + NI
        on = [w1 <= h <= w1_end or h >= w2 for h in (2 * j, 2 * j + 1)]
        nw = min(MAX_WR[1 - short], qs[j] - wn) if on[0] else 0
        nm = min(MAX_MID, qs[j] - wn - nw) if (on[1] and not short) else 0
        assert wn + nw + nm <= qs[j]
        tab += [rn, nr, wn, nw, nm]
        rn += nr
        wn += nw + nm
    assert rn == NQ and wn == NQ - 1
    return tab


def _comb(terms, get):
    v = get(terms[0][0])
    for q, s in terms[1:]:
        v = v + get(q) if s > 0 else v - get(q)
    return v


def _quadrants(a):
    h, w = a.shape[0] // 2, a.shape[1] // 2
    return a[:h, :w], a[:h, w:], a[h:, :w], a[h:, w:]


def _pack(a):
    return pltpu.bitcast(a.astype(BF16), I32)


def _unpack(a):
    return pltpu.bitcast(a, BF16)


class _Acc:
    def __init__(self, n):
        self.left, self.pos, self.neg = n, None, None

    def add(self, s, v):
        self.left -= 1
        if self.pos is not None:
            self.pos = self.pos + v if s > 0 else self.pos - v
        elif s > 0:
            self.pos = v if self.neg is None else v - self.neg
        else:
            self.neg = v if self.neg is None else self.neg + v
        return self.left == 0


def _prepare(w_ref, b_ref, wf_ref, sa_ref, wtail_ref, bias_ref):
    brow = b_ref[...].astype(F32).reshape(1, D)
    for j in range(5):
        if j < 4:
            blk = w_ref[:, 128 * j:128 * j + 128].astype(F32)
            bj = brow[:, 128 * j:128 * j + 128]
        else:
            blk = jnp.concatenate(
                [w_ref[:, 512:D].astype(F32), jnp.zeros((D, 64), F32)], axis=1)
            bj = jnp.concatenate([brow[:, 512:D], jnp.zeros((1, 64), F32)], axis=1)
        wf_ref[j, 0:D] = blk
        wf_ref[j, D:640] = jnp.broadcast_to(bj, (640 - D, 128))
    for j in range(5):
        v = [wf_ref[j, pl.ds(i, D // 4, stride=4), :] for i in range(4)]
        m = [jnp.abs(a) for a in v]
        hi1, lo1 = jnp.maximum(m[0], m[1]), jnp.minimum(m[0], m[1])
        hi2, lo2 = jnp.maximum(m[2], m[3]), jnp.minimum(m[2], m[3])
        thr = jnp.maximum(jnp.minimum(hi1, hi2), jnp.maximum(lo1, lo2))
        for i in range(4):
            wf_ref[j, pl.ds(i, D // 4, stride=4), :] = v[i] * (m[i] >= thr).astype(F32)
    wt = jnp.concatenate(
        [wf_ref[j].T if j < 4 else wf_ref[j].T[:64] for j in range(5)], axis=0)
    last = wt[:, 512:640]
    low = lax.broadcasted_iota(I32, last.shape, 1) < 64
    bias_ref[...] = jnp.where(low, pltpu.roll(last, 64, 1), last)
    wtail_ref[...] = _pack(last)
    a0 = _quadrants(wt[:, 0:512])
    for r in range(7):
        a1 = _quadrants(_comb(AT[r], lambda q: a0[q]))
        for t in range(7):
            sa_ref[7 * r + t] = _pack(_comb(AT[t], lambda u: a1[u]))


def _group(x_ref, o_ref, c0, nxt, first, pend, sa_ref, wtail_ref, bias_ref, done=None):
    def direct(r, t):
        return len(BT[r]) == 1 and len(BT[t]) == 1

    def tile(ref, c, q, u):
        k, j = 2 * (q // 2) + u // 2, 2 * (q % 2) + u % 2
        return ref[128 * k:128 * k + 128, pl.ds(c + 128 * j, 128)]

    def xop(r, ref, c):
        cache = {}

        def gx(q, u):
            if (q, u) not in cache:
                cache[(q, u)] = tile(ref, c, q, u).astype(F32)
            return cache[(q, u)]

        b1 = [_comb(BT[r], lambda q: gx(q, u)) for u in range(4)]
        for t in range(7):
            if not direct(r, t):
                pend[t] = _comb(BT[t], lambda u: b1[u]).astype(BF16)

    acc = {(q, u): _Acc(NT[q] + 1) for q in range(4) for u in range(4)}

    def put(q, u, s, v):
        if acc[(q, u)].add(s, v):
            r0 = 288 * (q // 2) + 144 * (u // 2)
            cc = 256 * (q % 2) + 128 * (u % 2)
            o_ref[r0:r0 + 144, pl.ds(c0 + cc, 128)] = acc[(q, u)].pos.astype(BF16)
            if done is not None and all(acc[(q, v)].left == 0 for v in range(4)):
                done(288 * (q // 2), c0 + 256 * (q % 2))

    def tails(pos):
        for j, p in TAIL_AT.items():
            if p == pos:
                t = jnp.dot(_unpack(wtail_ref[...])[:, 0:64],
                            x_ref[512:D, pl.ds(c0 + 128 * j, 128)],
                            preferred_element_type=F32) + bias_ref[...]
                for i in range(4):
                    put(2 * (i // 2) + j // 2, 2 * (i % 2) + j % 2, 1, t[144 * i:144 * i + 144])

    if first:
        xop(ORDER1[0], x_ref, c0)
    tails(-1)
    for pos, r in enumerate(ORDER1):
        c = [_Acc(NT[u]) for u in range(4)]
        for t in ORDER2:
            sb = tile(x_ref, c0, BT[r][0][0], BT[t][0][0]) if direct(r, t) else pend.pop(t)
            m = jnp.dot(_unpack(sa_ref[7 * r + t]), sb, preferred_element_type=F32)
            for u, s in CT[t]:
                if c[u].add(s, m):
                    for q, s1 in CT[r]:
                        put(q, u, s1, c[u].pos)
        if pos + 1 < 7:
            xop(ORDER1[pos + 1], x_ref, c0)
        elif nxt is not None:
            xop(ORDER1[0], nxt[0], nxt[2])
        tails(pos)


def _kernel(x_hbm, w_hbm, b_hbm, o_hbm, xbuf, obuf, w_ref, b_ref, wf_ref, sa_ref,
            wtail_ref, bias_ref, tab, rsem, wsem, csem):
    def rd(q):
        s = q & (NI - 1)
        src = x_hbm.at[q >> 2, :, pl.ds(pl.multiple_of((q & 3) * QW, QW), QW)]
        return pltpu.make_async_copy(src, xbuf.at[s], rsem.at[s])

    def wr(q, c0):
        dst = o_hbm.at[q >> 2, :, pl.ds(pl.multiple_of((q & 3) * QW + c0, 256), 256)]
        return pltpu.make_async_copy(obuf.at[q, :, pl.ds(c0, 256)], dst, wsem.at[0])

    cw = pltpu.make_async_copy(w_hbm, w_ref, csem.at[0])
    cb = pltpu.make_async_copy(b_hbm, b_ref, csem.at[1])
    cw.start()
    cb.start()
    rd(0).start()
    for i, v in enumerate(_dma_plan()):
        tab[i] = v
    cw.wait()
    cb.wait()
    rd(1).start()
    rd(2).start()
    _prepare(w_ref, b_ref, wf_ref, sa_ref, wtail_ref, bias_ref)
    for q in range(3, NINIT):
        rd(q).start()

    def writes(q0, n, nmax):
        for t in range(nmax):
            for c0 in range(0, QW, 256):
                @pl.when(t < n)
                def _():
                    wr(jnp.minimum(q0 + t, NQ - 1), c0).start()

    def rnd(nq, max_rd, max_wr):
        def body(_, carry):
            j, q = carry
            for k in range(nq):
                rd(q + k).wait()
            r0, nr, w0, nw, nm = [tab[5 * j + i] for i in range(5)]
            writes(w0, nw, max_wr)

            def last_quad_piece(row, col):
                @pl.when(q == NQ - 1)
                def _():
                    pltpu.make_async_copy(
                        obuf.at[NQ - 1, pl.ds(row, 288), pl.ds(col, 256)],
                        o_hbm.at[NQ // 4 - 1, pl.ds(row, 288), pl.ds(3 * QW + col, 256)],
                        wsem.at[0]).start()

            gs = [(xbuf.at[(q + k) & (NI - 1)], obuf.at[q + k], c0)
                  for k in range(nq) for c0 in range(0, QW, 512)]
            pend = {}
            for gi, (xv, ov, c0) in enumerate(gs):
                if nq > 1 and gi == nq:
                    writes(w0 + nw, nm, MAX_MID)
                nxt = gs[gi + 1] if gi + 1 < len(gs) else None
                _group(xv, ov, c0, nxt, gi == 0, pend, sa_ref, wtail_ref, bias_ref,
                       last_quad_piece if (nq == 1 and gi == 1) else None)
                if nq == 1 and gi == 0:
                    for c1 in (0, 256):
                        @pl.when(q == NQ - 1)
                        def _():
                            wr(NQ - 1, c1).start()
            for t in range(max_rd):
                @pl.when(t < nr)
                def _():
                    rd(jnp.minimum(r0 + t, NQ - 1)).start()
            return j + 1, q + nq
        return body

    def phase(ph, carry):
        carry = lax.fori_loop(0, jnp.where(ph == 0, NA0, NA1), rnd(1, MAX_RD[0], MAX_WR[0]), carry)
        nb = (NQ - NA0 - NA1) // NB
        return lax.fori_loop(0, jnp.where(ph == 0, nb, 0),
                             rnd(NB, MAX_RD[1], MAX_WR[1]), carry)

    lax.fori_loop(0, 2, phase, (jnp.int32(0), jnp.int32(0)))
    pltpu.make_async_copy(obuf, obuf, wsem.at[0]).wait()


@jax.jit
def pallas_standalone__structured_sparse_n_m__ragged_kernel(
    x: jax.Array,
    w: jax.Array,
    b: jax.Array,
):
    B, S, _ = x.shape
    assert x.shape == (16, 4096, D) and w.shape == (D, D) and b.shape == (D,)
    any_spec = pl.BlockSpec(memory_space=pl.ANY)
    out_t = pl.pallas_call(
        _kernel,
        in_specs=[any_spec] * 3,
        out_specs=any_spec,
        out_shape=jax.ShapeDtypeStruct((B, D, S), x.dtype),
        scratch_shapes=[
            pltpu.VMEM((NI, D, QW), BF16),
            pltpu.VMEM((NQ, D, QW), BF16),
            pltpu.VMEM((D, D), BF16),
            pltpu.VMEM((D,), BF16),
            pltpu.VMEM((5, 640, 128), F32),
            pltpu.VMEM((49, 72, 128), I32),
            pltpu.VMEM((D // 2, 128), I32),
            pltpu.VMEM((D, 128), F32),
            pltpu.SMEM((len(_dma_plan()),), I32),
            pltpu.SemaphoreType.DMA((NI,)),
            pltpu.SemaphoreType.DMA((1,)),
            pltpu.SemaphoreType.DMA((2,)),
        ],
        compiler_params=pltpu.CompilerParams(
            vmem_limit_bytes=124 * 1024 * 1024, disable_bounds_checks=True),
    )(jnp.swapaxes(x, 1, 2), w, b)
    return jnp.swapaxes(out_t, 1, 2)
```
